```python
import jax
import jax.numpy as jnp

def _softmax(x, axis=-1):
    return jax.nn.softmax(x, axis=axis)
def _gelu(x):
    return jax.nn.gelu(x, approximate=True)
def _silu(x):
    return jax.nn.silu(x)
def _sigmoid(x):
    return jax.nn.sigmoid(x)
def _layernorm(x, axis=-1, eps=1e-5):
    m = jnp.mean(x, axis=axis, keepdims=True)
    v = jnp.var(x, axis=axis, keepdims=True)
    return (x - m) / jnp.sqrt(v + eps)
def _scatter_add(tgt, idx, src, axis=0):
    return tgt.at[idx].add(src)
def _segment_sum(src, seg, n):
    return jax.ops.segment_sum(src, seg, n)
class _Rng:
    def __init__(self, key):
        self._k = key
    def _next(self):
        self._k, sub = jax.random.split(self._k)
        return sub
    def normal(self, shape):
        return jax.random.normal(self._next(), shape, dtype=jnp.bfloat16)
    def randint(self, lo, hi, shape):
        return jax.random.randint(self._next(), shape, lo, hi, dtype=jnp.int32)
    def uniform(self, shape, lo=0.0, hi=1.0):
        return jax.random.uniform(self._next(), shape, jnp.bfloat16, lo, hi)
    def permutation(self, n):
        return jax.random.permutation(self._next(), n)


kernel_name = 'standalone__mha_softmax__near_ridge'

def _fwd_setup_inputs():
    _rng = _Rng(jax.random.key(int.from_bytes(__import__("os").urandom(4), "little")))
    _w = (lambda a: (lambda t: t.astype(jnp.bfloat16) if jnp.issubdtype(t.dtype, jnp.floating) else t)(jnp.asarray(a)))
    B, H, Sq, Sk, D = 16, 32, 384, 1024, 128
    return {
        "q": _w((lambda *s: _rng.normal(s) * 0.05)(B, H, Sq, D)),
        "k": _w((lambda *s: _rng.normal(s) * 0.05)(B, H, Sk, D)),
        "v": _w((lambda *s: _rng.normal(s) * 0.05)(B, H, Sk, D)),
    }

def _fwd_reference(q, k, v):
    scale = q.shape[-1] ** -0.5
    scores = jnp.einsum("bhqd,bhkd->bhqk", q, k) * scale
    p = _softmax(scores, axis=-1)
    return jnp.einsum("bhqk,bhkd->bhqd", p, v)


def setup_inputs():
    _inp = _fwd_setup_inputs()
    _gk = jax.random.fold_in(jax.random.key(int.from_bytes(__import__("os").urandom(4), "little")), 2**31 - 1)
    _shapes = [[16, 32, 384, 128]]
    _dtypes = ['bfloat16']
    _gks = jax.random.split(_gk, len(_shapes))
    _gs = [jax.random.normal(k, s, dtype=jnp.dtype(d)) * 0.05 for k, s, d in zip(_gks, _shapes, _dtypes)]
    _inp["grad_out"] = _gs[0]
    return _inp

def reference(q, k, v, grad_out):
    _const = dict()
    def _f(*_d):
        return _fwd_reference(**{'q': _d[0], 'k': _d[1], 'v': _d[2], **_const})
    _out, _vjp = jax.vjp(_f, q, k, v)
    _grads = _vjp(grad_out)
    _out0 = jnp.asarray(_out)
    return (_out0, *[jnp.asarray(_g) for _g in _grads])
```

```python
import functools, math
import jax, jax.numpy as jnp
from jax import lax
import jax.experimental.pallas as pl
import jax.experimental.pallas.tpu as pltpu

F32, BF16, U32 = jnp.float32, jnp.bfloat16, jnp.uint32
NT = (((1,), (1,)), ((), ()))
NN = (((1,), (0,)), ((), ()))
dg = lambda a, b, d: lax.dot_general(a, b, d, preferred_element_type=F32)
pk = lambda x: pltpu.bitcast(x.astype(BF16), U32)
upk = lambda x: pltpu.bitcast(x, BF16)

def zero_tok(x):
    u = pltpu.bitcast(x, U32)
    return pltpu.bitcast(lax.shift_right_logical(lax.shift_right_logical(u, jnp.uint32(31)), jnp.uint32(1)), F32)

def make(hb=2, CH=256, xt=False, nbuf=2, G=2, lo0=0.15, hi0=0.8, lo=0.0, hi=1.0):
    def kernel(q_ref, k_ref, v_ref, g_ref, o_ref, dq_ref, dk_ref, dv_ref, *scr):
        Sq, D = q_ref.shape[1:]; Sk = k_ref.shape[1]
        z = lax.shift_right_logical(pl.program_id(0), 20)
        zb = lax.shift_right_logical(pl.program_id(0), 21)
        s_scr, e_scr, ds_scr, t_scr = [[r.at[z] for r in scr[i * nbuf:(i + 1) * nbuf]] for i in range(4)]
        s_ld = [r.at[zb] for r in scr[:nbuf]]
        nc = Sk // CH
        scale = D ** -0.5
        c2 = scale * math.log2(math.e)
        rows = lambda c: pl.ds(c * CH, CH)
        hrows = lambda c: pl.ds(c * CH // 2, CH // 2)
        st = [dict() for _ in range(hb)]
        def tr(ref, h, slot):
            if not xt: return ref[h].T
            t_scr[h % nbuf][slot] = pk(ref[h].T)
            return upk(t_scr[h % nbuf][slot])
        def S(h):
            q = q_ref[h]; b = h % nbuf
            m8 = None; toks = []
            for c in range(nc):
                s = dg(k_ref[h, rows(c), :], q, NT)
                for j in range(3):
                    if (3 * c + j) % 4 == 0:
                        toks += [s[8 * r:8 * r + 8, 128 * j:128 * (j + 1)] for r in range(CH // 8)]
                s = s * c2
                s_scr[b][rows(c), :] = s
                mc = jnp.max(s.reshape(CH // 8, 8, Sq), axis=0)
                m8 = mc if m8 is None else jnp.maximum(m8, mc)
            st[h]["m"] = jnp.max(m8, axis=0, keepdims=True)
            return toks
        def X(h, toks, lo, hi):
            b = h % nbuf
            m8 = jnp.broadcast_to(st[h]["m"], (8, Sq))
            l8 = None
            n = Sk // 16
            for r in range(n):
                if r % G == 0:
                    t = zero_tok(toks[min(len(toks) - 1, int(len(toks) * (lo + (hi - lo) * (r + G) / n)))])
                    t = jnp.concatenate([t] * (Sq // 128), axis=1)
                e0 = jnp.exp2(s_ld[b][pl.ds(r * 16, 8), :] - m8) + t
                e1 = jnp.exp2(s_ld[b][pl.ds(r * 16 + 8, 8), :] - m8)
                e_scr[b][pl.ds(r * 8, 8), :] = pk(jnp.concatenate([e0, e1], axis=0))
                lc = e0 + e1
                l8 = lc if l8 is None else l8 + lc
            st[h]["linv"] = 1.0 / jnp.sum(l8, axis=0, keepdims=True)
        def O(h):
            linv = st[h]["linv"]; b = h % nbuf
            ot = dg(tr(v_ref, h, 0), upk(e_scr[b][...]), NN) * linv
            o_ref[h] = ot.T.astype(BF16)
            gt = g_ref[h].T.astype(F32) * linv
            st[h]["gs"] = gt.astype(BF16)
            gs2 = (gt * scale).astype(BF16)
            st[h]["gs2"] = gs2
            st[h]["delta"] = jnp.sum(gs2.astype(F32) * ot, axis=0, keepdims=True)
        def dV(h):
            for c in range(nc):
                dv_ref[h, rows(c), :] = dg(upk(e_scr[h % nbuf][hrows(c), :]), st[h]["gs"], NT).astype(BF16)
        def dP(h):
            b = h % nbuf
            for c in range(nc):
                dp = dg(v_ref[h, rows(c), :], st[h]["gs2"], NN) - st[h]["delta"]
                ds_scr[b][hrows(c), :] = pk(upk(e_scr[b][hrows(c), :]).astype(F32) * dp)
        def dQ(h):
            dqt = dg(tr(k_ref, h, 1), upk(ds_scr[h % nbuf][...]), NN)
            dq_ref[h] = dqt.T.astype(BF16)
        def dK(h):
            q = q_ref[h]; toks = []
            for c in range(nc):
                dk = dg(upk(ds_scr[h % nbuf][hrows(c), :]), q, NN)
                dk_ref[h, rows(c), :] = dk.astype(BF16)
                if c % 4 != 2: toks += [dk[8 * r:8 * r + 8] for r in range(CH // 8)]
            return toks
        S(0)
        X(0, S(1), lo0, hi0)
        for h in range(hb):
            O(h)
            if h > 0 and h + 1 < hb: S(h + 1)
            dV(h); dP(h)
            if h + 1 < hb:
                X(h + 1, dK(h), lo, hi); dQ(h)
            else:
                dQ(h); dK(h)
    @jax.jit
    def f(q, k, v, g):
        B, H, Sq, D = q.shape; Sk = k.shape[2]; BH = B * H
        q, k, v, g = [x.reshape(BH, x.shape[2], D) for x in (q, k, v, g)]
        qs = pl.BlockSpec((hb, Sq, D), lambda i: (i, 0, 0)); ks = pl.BlockSpec((hb, Sk, D), lambda i: (i, 0, 0))
        sq = jax.ShapeDtypeStruct((BH, Sq, D), BF16); sk = jax.ShapeDtypeStruct((BH, Sk, D), BF16)
        o, dq, dk, dv = pl.pallas_call(kernel, grid=(BH // hb,), in_specs=[qs, ks, ks, qs], out_specs=[qs, qs, ks, ks],
            out_shape=[sq, sq, sk, sk], name="mha",
            scratch_shapes=[pltpu.VMEM((1, Sk, Sq), F32)] * nbuf + [pltpu.VMEM((1, Sk // 2, Sq), U32)] * (2 * nbuf) + [pltpu.VMEM((1, 2, D // 2, Sk), U32)] * nbuf,
            compiler_params=pltpu.CompilerParams(dimension_semantics=("parallel",), vmem_limit_bytes=100 << 20))(q, k, v, g)
        return o.reshape(B, H, Sq, D), dq.reshape(B, H, Sq, D), dk.reshape(B, H, Sk, D), dv.reshape(B, H, Sk, D)
    return f

_impl = make(hb=4)

@jax.jit
def pallas_standalone__mha_softmax__near_ridge_kernel(q, k, v, grad_out):
    return _impl(q, k, v, grad_out)
```

```python
import functools, math
import jax, jax.numpy as jnp
from jax import lax
import jax.experimental.pallas as pl
import jax.experimental.pallas.tpu as pltpu

F32, BF16, U32 = jnp.float32, jnp.bfloat16, jnp.uint32
NT = (((1,), (1,)), ((), ()))
NN = (((1,), (0,)), ((), ()))
dg = lambda a, b, d: lax.dot_general(a, b, d, preferred_element_type=F32)
pk = lambda x: pltpu.bitcast(x.astype(BF16), U32)
upk = lambda x: pltpu.bitcast(x, BF16)

def restore(x):
    return pltpu.bitcast(pltpu.bitcast(x.astype(F32), U32), F32).astype(BF16)

def zero_tok(x):
    u = pltpu.bitcast(x, U32)
    return pltpu.bitcast(lax.shift_right_logical(lax.shift_right_logical(u, jnp.uint32(31)), jnp.uint32(1)), F32)

def ttok(x):
    u = pltpu.bitcast(x, U32)
    return zero_tok(functools.reduce(jnp.bitwise_or, [u[64 * j + 56:64 * j + 64] for j in range(u.shape[0] // 64)]))

def make(U=4, CH=256, G=2, lo=0.0, hi=1.0, lo2=0.0, hi2=0.93, DC=256, NAT=2, rl=True):
    ld = restore if rl else (lambda x: x)
    def kernel(*refs):
        hin, hout, scr = refs[:4], refs[4:8], refs[8:]
        BH, Sq, D = hin[0].shape; Sk = hin[1].shape[1]
        ib, xb, ob = scr[0:4], scr[4:6], scr[6:10]
        s_raw, pc_raw, dc_raw, isem, osem = scr[10:]
        NG = BH // U
        nc = Sk // CH
        scale = D ** -0.5
        c2 = scale * math.log2(math.e)
        rows = lambda c: pl.ds(c * CH, CH)
        hrows = lambda c: pl.ds(c * CH // 2, CH // 2)
        icp = lambda a, i, p: pltpu.make_async_copy(hin[a].at[pl.ds(i * U, U)], ib[a].at[p], isem.at[2 * a + p])
        xcp = lambda a, n, p: pltpu.make_async_copy(hin[a].at[n], xb[a].at[p], isem.at[8 + 2 * a + p])
        ocp = lambda a, n, p, h: pltpu.make_async_copy(ob[a].at[p, h], hout[a].at[n], osem.at[2 * a + p])
        owait = lambda a, p: pltpu.make_async_copy(ob[a].at[p], ob[a].at[p], osem.at[2 * a + p]).wait()
        def fetch(i, p):
            cps = [icp(a, i, p) for a in range(4)]
            return cps + [xcp(a, jnp.minimum(i * U + U, BH - 1), p) for a in range(2)]

        def phases(i, p):
            q_b, k_b, v_b, g_b = [[r.at[p, h] for h in range(U)] for r in ib]
            q_b.append(xb[0].at[p]); k_b.append(xb[1].at[p])
            o_b, dq_b, dk_b, dv_b = [[r.at[p, h] for h in range(U)] for r in ob]
            z = lax.shift_right_logical(i, 20)
            zb = lax.shift_right_logical(i, 21)
            s_st, s_ld = s_raw.at[z], s_raw.at[zb]
            pc, dc = pc_raw.at[z], dc_raw.at[z]
            blk = lambda ref, j, r0=0, nr=Sk // 4: upk(ref[pl.ds(r0, nr), pl.ds(128 * j, 128)])
            st = [dict(t=[]) for _ in range(U + 1)]
            HK = Sk // 2
            pick = lambda toks, f: zero_tok(toks[min(len(toks) - 1, int(len(toks) * f))])
            vregs = lambda x: [x[8 * r:8 * r + 8] for r in range(x.shape[0] // 8)]
            paced = lambda x, t: x if t is None else jnp.concatenate([x[:8] + jnp.concatenate([t] * (x.shape[1] // 128), axis=1), x[8:]], axis=0)
            def bcomb(u, l):
                b11, b12, b21, b22 = u[:, :128], u[:, 128:], l[:, :128], l[:, 128:]
                t1 = b12 - b11; t2 = b22 - t1; t3 = b22 - b12; t4 = t2 - b21
                return [b11, b21, b22, t4, t1, t2, t3, b12]
            def prob1(x, cb):
                at = x.T; af = at.astype(F32)
                s1 = af[64:, :HK] + af[64:, HK:]; s2 = s1 - af[:64, :HK]; s3 = af[:64, :HK] - af[64:, :HK]; s4 = af[:64, HK:] - s2
                a = [at[:64, :HK], at[:64, HK:], s4.astype(BF16), at[64:, HK:], s1.astype(BF16), s2.astype(BF16), s3.astype(BF16)]
                x0 = dg(at[:, :HK], blk(cb, 8), NN)
                x1 = dg(at[:, HK:], blk(cb, 9), NN)
                toks = vregs(x0) + vregs(x1)
                m = {}
                for r in (0, 1, 5, 6, 4, 2, 3):
                    m[r] = dg(a[r], blk(cb, r), NN); toks += vregs(m[r])
                u2 = m[0] + m[5]; u3 = u2 + m[6]
                c11 = m[0] + m[1]; c12 = u2 + m[4] + m[2]; c21 = u3 - m[3]; c22 = u3 + m[4]
                return jnp.concatenate([jnp.concatenate([c11, c21], axis=0), jnp.concatenate([c12, c22], axis=0), x0 + x1], axis=1), toks
            def prob2(xt, cb, out, nt=4):
                xf = xt[:, :256].astype(F32)
                z5 = xf[:64, 128:] + xf[64:, 128:]; z6 = z5 + xf[64:, :128]; z1 = z6 + xf[:64, :128]; z7 = xf[64:, :128] + xf[64:, 128:]
                zz = [z1.astype(BF16), xt[:64, :128], xt[:64, 128:256], xt[64:, :128], z5.astype(BF16), z6.astype(BF16), z7.astype(BF16)]
                toks, tt = [], []
                for t in range(nt):
                    n = {}
                    y0 = dg(xt[:, 256:], blk(cb, 8, 64 * t, 64), NT)
                    y1 = dg(xt[:, 256:], blk(cb, 9, 64 * t, 64), NT)
                    for r in (2, 5, 4, 1, 3, 6, 0):
                        n[r] = dg(zz[r], blk(cb, r, 64 * t, 64), NT)
                    toks += vregs(n[2]) + vregs(n[4]) + vregs(n[0])
                    w = n[5] - n[2]; y = w + n[4]
                    l = jnp.concatenate([n[1] + n[2], y - n[3]], axis=0) + y1
                    u = jnp.concatenate([n[0] + n[6] - w, y - n[6]], axis=0) + y0
                    for base, val in ((HK, l), (0, u)):
                        val = val.astype(BF16).T
                        out[pl.ds(base + 128 * t, 128), :] = restore(val)
                        tt.append(pltpu.bitcast(val, U32)[56:64])
                return toks, zero_tok(functools.reduce(jnp.bitwise_or, tt))
            def S(h):
                q = ld(q_b[h][...])
                m8 = None
                for c in range(nc):
                    s = dg(ld(k_b[h][rows(c), :]), q, NT) * c2
                    s_st[rows(c), :] = s
                    mc = jnp.max(s.reshape(CH // 8, 8, Sq), axis=0)
                    m8 = mc if m8 is None else jnp.maximum(m8, mc)
                st[h]["m"] = jnp.max(m8, axis=0, keepdims=True)
            def X1(h, toks):
                m8 = jnp.broadcast_to(st[h]["m"], (8, Sq))
                l8 = None
                n = Sk // 8
                for r in range(n):
                    e = jnp.exp2(s_ld[pl.ds(r * 8, 8), :] - m8)
                    if toks and r % (2 * G) == 0:
                        e = e + jnp.concatenate([pick(toks, lo + (hi - lo) * (r + 2 * G) / n)] * 3, axis=1)
                    l8 = e if l8 is None else l8 + e
                st[h]["m2"] = st[h]["m"] + jnp.log2(jnp.sum(l8, axis=0, keepdims=True))
            def X2(h, toks):
                m16 = jnp.broadcast_to(st[h]["m2"], (16, Sq))
                n = HK // 16
                for r in range(n):
                    t = pick(toks, lo2 + (hi2 - lo2) * (r + 1) / n) if toks else None
                    u = paced(jnp.exp2(s_ld[pl.ds(r * 16, 16), :] - m16), t)
                    l = paced(jnp.exp2(s_ld[pl.ds(HK + r * 16, 16), :] - m16), t)
                    pc[pl.ds(r * 8, 8), :] = pk(jnp.concatenate(bcomb(u[:, :256], l[:, :256]) + [u[:, 256:], l[:, 256:]], axis=1))
            def O(h):
                ot, toks = prob1(ld(v_b[h][...]), pc)
                o = ot.astype(BF16).T
                o_b[h][...] = restore(o)
                gt = ld(g_b[h][...]).T
                st[h]["gt"] = gt
                g2 = (gt.astype(F32) * scale).astype(BF16)
                st[h]["g2"] = g2
                t = functools.reduce(jnp.add, [ttok(o)] + (st[h - 1]["t"] if h > 0 else []))
                st[h]["delta"] = jnp.sum(g2.astype(F32) * ot, axis=0, keepdims=True) + jnp.concatenate([t[0:1]] * 3, axis=1)
            def dV(h):
                toks, t = prob2(st[h]["gt"], pc, dv_b[h])
                st[h]["t"].append(t)
                return toks
            def dP(h):
                g2, delta = st[h]["g2"], st[h]["delta"]
                for c in range(2):
                    dp = [dg(ld(v_b[h][pl.ds(b + c * 256, 256), :]), g2[:, 256:], NN) - delta[:, 256:] for b in (0, HK)]
                    hr = pl.ds(c * 128, 128)
                    dc[hr, pl.ds(1024, 256)] = pk(upk(pc[hr, pl.ds(1024, 256)]).astype(F32) * jnp.concatenate(dp, axis=1))
                for c in range(HK // DC):
                    hr = pl.ds(c * DC // 2, DC // 2)
                    pb = lambda j: blk(pc, j, c * DC // 2, DC // 2).astype(F32)
                    u = (dg(ld(v_b[h][pl.ds(c * DC, DC), :]), g2[:, :256], NN) - delta[:, :256]) * jnp.concatenate([pb(0), pb(7)], axis=1)
                    l = (dg(ld(v_b[h][pl.ds(HK + c * DC, DC), :]), g2[:, :256], NN) - delta[:, :256]) * jnp.concatenate([pb(1), pb(2)], axis=1)
                    nb = 8 if h == U - 1 and (c + 1) * DC > (4 - NAT) * 128 else 7
                    dc[hr, pl.ds(0, 128 * nb)] = pk(jnp.concatenate(bcomb(u, l)[:nb], axis=1))
            def dQ(h):
                dqt, toks = prob1(ld(k_b[h][...]), dc)
                dq = dqt.astype(BF16).T
                dq_b[h][...] = restore(dq)
                st[h]["t"].append(ttok(dq))
                return toks
            def dK(h):
                q = ld(q_b[h][...])
                nt = 4 - NAT if h == U - 1 else 4
                toks, t = prob2(q.T, dc, dk_b[h], nt)
                st[h]["t"].append(t)
                for t in range(nt, 4):
                    for base, js in ((0, (0, 7, 8)), (HK, (1, 2, 9))):
                        dk = dg(jnp.concatenate([blk(dc, j, 64 * t, 64) for j in js], axis=1), q, NN)
                        toks += vregs(dk)[::2]
                        if t == 3 and base: dk = jnp.concatenate([dk[:120], dk[120:] + functools.reduce(jnp.add, st[h]["t"])], axis=0)
                        dk_b[h][pl.ds(base + 128 * t, 128), :] = dk.astype(BF16)
                return toks
            return S, X1, X2, O, dV, dP, dQ, dK

        for a in range(2): xcp(a, 0, 1).start()
        for c in fetch(0, 0): c.start()
        for a in range(2): xcp(a, 0, 1).wait()
        S, X1, X2 = phases(pl.program_id(0), 1)[:3]
        S(U); X1(U, None); X2(U, None)

        def body(i, carry):
            p = lax.rem(i, 2)
            for c in fetch(i, p): c.wait()
            @pl.when(i > 1)
            def _():
                for a in range(4): owait(a, p)
            @pl.when(i + 1 < NG)
            def _():
                for c in fetch(i + 1, 1 - p): c.start()
            S, X1, X2, O, dV, dP, dQ, dK = phases(i, p)
            for h in range(U):
                S(h + 1); O(h)
                X1(h + 1, dV(h))
                dP(h)
                X2(h + 1, dQ(h) + dK(h))
                for a in range(4): ocp(a, i * U + h, p, h).start()
            return carry
        lax.fori_loop(0, NG, body, 0)
        for p in range(2):
            for a in range(4): owait(a, p)

    @jax.jit
    def f(q, k, v, g):
        B, H, Sq, D = q.shape; Sk = k.shape[2]; BH = B * H
        q, k, v, g = [x.reshape(BH, x.shape[2], D) for x in (q, k, v, g)]
        sq = jax.ShapeDtypeStruct((BH, Sq, D), BF16); sk = jax.ShapeDtypeStruct((BH, Sk, D), BF16)
        bq = [pltpu.VMEM((2, U, Sq, D), BF16)]; bk = [pltpu.VMEM((2, U, Sk, D), BF16)]
        bx = [pltpu.VMEM((2, Sq, D), BF16), pltpu.VMEM((2, Sk, D), BF16)]
        cb = pltpu.VMEM((1, Sk // 4, 1280), U32)
        anyspec = pl.BlockSpec(memory_space=pl.ANY)
        o, dq, dk, dv = pl.pallas_call(kernel, grid=(1,), in_specs=[anyspec] * 4, out_specs=[anyspec] * 4,
            out_shape=[sq, sq, sk, sk], name="mha",
            scratch_shapes=bq + bk + bk + bq + bx + bq + bq + bk + bk + [pltpu.VMEM((1, Sk, Sq), F32), cb, cb,
                pltpu.SemaphoreType.DMA((12,)), pltpu.SemaphoreType.DMA((8,))],
            compiler_params=pltpu.CompilerParams(dimension_semantics=("arbitrary",), vmem_limit_bytes=100 << 20))(q, k, v, g)
        return o.reshape(B, H, Sq, D), dq.reshape(B, H, Sq, D), dk.reshape(B, H, Sk, D), dv.reshape(B, H, Sk, D)
    return f

_impl = make(U=4,rl=False)

@jax.jit
def pallas_standalone__mha_softmax__near_ridge_kernel(q, k, v, grad_out):
    return _impl(q, k, v, grad_out)
```

```python
import functools, math
import jax, jax.numpy as jnp
from jax import lax
import jax.experimental.pallas as pl
import jax.experimental.pallas.tpu as pltpu

F32, BF16, U32 = jnp.float32, jnp.bfloat16, jnp.uint32
NT = (((1,), (1,)), ((), ()))
NN = (((1,), (0,)), ((), ()))
dg = lambda a, b, d: lax.dot_general(a, b, d, preferred_element_type=F32)
pk = lambda x: pltpu.bitcast(x.astype(BF16), U32)
upk = lambda x: pltpu.bitcast(x, BF16)

def restore(x):
    return pltpu.bitcast(pltpu.bitcast(x.astype(F32), U32), F32).astype(BF16)

def zero_tok(x):
    u = pltpu.bitcast(x, U32)
    return pltpu.bitcast(lax.shift_right_logical(lax.shift_right_logical(u, jnp.uint32(31)), jnp.uint32(1)), F32)

def make(U=6, U0=2, CH=256, G=4, NAT=2):
    def kernel(*refs):
        hin, hout = refs[:4], refs[4:8]
        ib, ob, ib0, ob0, s_raw, w_raw, pc_raw, pc_raw2, dc_raw, isem, osem = refs[8:]
        D = hin[0].shape[1]; Sk, Sq = s_raw.shape[1:]; BH = hin[0].shape[0] // Sq
        NG = (BH - U0) // U
        assert NG * U + U0 == BH
        nc = Sk // CH
        scale = D ** -0.5
        c2 = scale * math.log2(math.e)
        rows = lambda c: pl.ds(c * CH, CH)
        il, ol = (Sq, Sk, Sk, Sq), (Sq, Sq, Sk, Sk)
        ioff = lambda a, U: sum(il[j] * (U + (j < 2)) for j in range(a))
        hsl = lambda r, n, c, L: r.at[pl.ds(n * L if isinstance(n, int) else pl.multiple_of(n * L, 128), c * L)]
        icp = lambda buf, U, a, n, h, c, sem: pltpu.make_async_copy(hsl(hin[a], n, c, il[a]), buf.at[pl.ds(ioff(a, U) + h * il[a], c * il[a])], sem)
        oview = lambda buf, U, a, h: buf.at[pl.ds(U * sum(ol[:a]) + h * ol[a], ol[a])]
        wait_all = lambda buf, sem: pltpu.make_async_copy(buf, buf, sem).wait()
        def fetch(i, p):
            n = U0 + i * U
            for a in range(4): icp(ib.at[p], U, a, n, 0, U, isem.at[p]).start()
            for a in range(2): icp(ib.at[p], U, a, jnp.minimum(n + U, BH - 1), U, 1, isem.at[p]).start()

        def phases(i, ibuf, obuf, U, old=None):
            rtok = lambda a, h, r0: zero_tok(pltpu.bitcast(oview(old, U, a, h)[pl.ds(r0, 16), :], U32))
            q_b, k_b, v_b, g_b = [[ibuf.at[pl.ds(ioff(a, U) + h * il[a], il[a])] for h in range(U + (a < 2))] for a in range(4)]
            o_b, dq_b, dk_b, dv_b = [[oview(obuf, U, a, h) for h in range(U)] for a in range(4)]
            z = lax.shift_right_logical(i, 20)
            zb = lax.shift_right_logical(i, 21)
            s_st, s_ld = s_raw.at[z], s_raw.at[zb]
            w_st, w_ld = w_raw.at[z], w_raw.at[zb]
            pcs, dc = (pc_raw.at[z], pc_raw2.at[z]), dc_raw.at[z]
            blk = lambda ref, j, r0=0, nr=Sk // 4: upk(ref[pl.ds(r0, nr), pl.ds(128 * j, 128)])
            st = [dict(t=[]) for _ in range(U + 1)]
            HK = Sk // 2
            pick = lambda toks, f: zero_tok(toks[min(len(toks) - 1, int(len(toks) * f))])
            vregs = lambda x: [x[8 * r:8 * r + 8] for r in range(x.shape[0] // 8)]
            paced = lambda x, t: x if t is None else jnp.concatenate([x[:8] + jnp.concatenate([t] * (x.shape[1] // 128), axis=1), x[8:]], axis=0)
            def bcomb(u, l):
                b11, b12, b21, b22 = u[:, :128], u[:, 128:], l[:, :128], l[:, 128:]
                t1 = b12 - b11; t2 = b22 - t1; t3 = b22 - b12; t4 = t2 - b21
                return [b11, b21, b22, t4, t1, t2, t3, b12]
            def prob1(x, cb):
                at = x.T; af = at.astype(F32)
                s1 = af[64:, :HK] + af[64:, HK:]; s2 = s1 - af[:64, :HK]; s3 = af[:64, :HK] - af[64:, :HK]; s4 = af[:64, HK:] - s2
                a = [at[:64, :HK], at[:64, HK:], s4.astype(BF16), at[64:, HK:], s1.astype(BF16), s2.astype(BF16), s3.astype(BF16)]
                a += [None, at[:, :HK], at[:, HK:]]
                m, toks = {}, []
                for r in (0, 1, 5, 6, 4, 2, 3, 8, 9):
                    m[r] = dg(a[r], blk(cb, r), NN); toks += vregs(m[r])
                x0, x1 = m[8], m[9]
                u2 = m[0] + m[5]; u3 = u2 + m[6]
                c11 = m[0] + m[1]; c12 = u2 + m[4] + m[2]; c21 = u3 - m[3]; c22 = u3 + m[4]
                return jnp.concatenate([jnp.concatenate([c11, c21], axis=0), jnp.concatenate([c12, c22], axis=0), x0 + x1], axis=1), toks
            def prob2(xt, cb, out, nt=4):
                xf = xt[:, :256].astype(F32)
                z5 = xf[:64, 128:] + xf[64:, 128:]; z6 = z5 + xf[64:, :128]; z1 = z6 + xf[:64, :128]; z7 = xf[64:, :128] + xf[64:, 128:]
                zz = [z1.astype(BF16), xt[:64, :128], xt[:64, 128:256], xt[64:, :128], z5.astype(BF16), z6.astype(BF16), z7.astype(BF16)]
                toks, tt = [], []
                for t in range(nt):
                    n = {}
                    y0 = dg(xt[:, 256:], blk(cb, 8, 64 * t, 64), NT)
                    y1 = dg(xt[:, 256:], blk(cb, 9, 64 * t, 64), NT)
                    for r in (2, 5, 4, 1, 3, 6, 0):
                        n[r] = dg(zz[r], blk(cb, r, 64 * t, 64), NT)
                    toks += vregs(n[2]) + vregs(n[4]) + vregs(n[0])
                    w = n[5] - n[2]; y = w + n[4]
                    l = jnp.concatenate([n[1] + n[2], y - n[3]], axis=0) + y1
                    u = jnp.concatenate([n[0] + n[6] - w, y - n[6]], axis=0) + y0
                    for base, val in ((HK, l), (0, u)):
                        val = val.astype(BF16).T
                        out[pl.ds(base + 128 * t, 128), :] = restore(val)
                        tt.append(pltpu.bitcast(val, U32)[56:64])
                return toks, zero_tok(functools.reduce(jnp.bitwise_or, tt))
            def S(h):
                q = q_b[h][...]
                m8, toks = None, []
                for c in range(nc):
                    s = dg(k_b[h][rows(c), :], q, NT) * c2
                    s_st[rows(c), :] = s
                    if c < 3: toks += vregs(s[:, 128 * c:128 * c + 128])
                    mc = jnp.max(s.reshape(CH // 8, 8, Sq), axis=0)
                    m8 = mc if m8 is None else jnp.maximum(m8, mc)
                st[h]["m"] = jnp.max(m8, axis=0, keepdims=True)
                return toks
            def X1(h, toks):
                m8 = jnp.broadcast_to(st[h]["m"], (8, Sq))
                l8 = None
                n = Sk // 8
                for r in range(n):
                    e = jnp.exp2(s_ld[pl.ds(r * 8, 8), :] - m8)
                    if toks and r % (2 * G) == 0:
                        e = e + jnp.concatenate([pick(toks, (r + 2 * G) / n)] * 3, axis=1)
                    l8 = e if l8 is None else l8 + e
                st[h]["m2"] = st[h]["m"] + jnp.log2(jnp.sum(l8, axis=0, keepdims=True))
            def X2(h, toks):
                pc = pcs[h % 2]
                m16 = jnp.broadcast_to(st[h]["m2"], (16, Sq))
                n = HK // 16
                for r in range(n):
                    t = pick(toks, (r + 1) / n) if toks else None
                    if toks and r in (4, 16): t = t + st[h - 1]["t"][r // 16]
                    u = paced(jnp.exp2(s_ld[pl.ds(r * 16, 16), :] - m16), t)
                    l = paced(jnp.exp2(s_ld[pl.ds(HK + r * 16, 16), :] - m16), t)
                    pc[pl.ds(r * 8, 8), :] = pk(jnp.concatenate(bcomb(u[:, :256], l[:, :256]) + [u[:, 256:], l[:, 256:]], axis=1))
            def O(h):
                pc = pcs[h % 2]
                ot, toks = prob1(v_b[h][...], pc)
                o = ot.astype(BF16).T
                o_b[h][...] = restore(o)
                st[h]["t"].append(rtok(0, h, 0))
                return toks
            def dV(h):
                pc = pcs[h % 2]
                toks, t = prob2(st[h]["gt"], pc, dv_b[h])
                st[h]["t"].append(rtok(3, h, 0))
                return toks
            def dP(h):
                pc = pcs[h % 2]
                gt = g_b[h][...].T
                st[h]["gt"] = gt
                g2 = (g_b[h][...].astype(F32) * scale).astype(BF16)
                d8 = None
                for c in range(nc):
                    r0 = c * CH % HK
                    pb = jnp.concatenate([blk(pc, j, r0 // 2, CH // 2) for j in ((0, 7, 8) if c * CH < HK else (1, 2, 9))], axis=1)
                    w = dg(v_b[h][rows(c), :], g2, NT) * pb.astype(F32)
                    w_st[rows(c), :] = w
                    wc = jnp.sum(w.reshape(CH // 8, 8, Sq), axis=0)
                    d8 = wc if d8 is None else d8 + wc
                delta = jnp.sum(d8, axis=0, keepdims=True)
                if h > 0: delta = delta + jnp.concatenate([functools.reduce(jnp.add, st[h - 1]["t"])[0:1]] * 3, axis=1)
                st[h]["delta"] = delta
            def Y(h, toks):
                pc = pcs[h % 2]
                d16 = jnp.broadcast_to(st[h]["delta"], (16, Sq))
                n = HK // 16
                for r in range(n):
                    t = pick(toks, (r + 1) / n)
                    pb = lambda js: jnp.concatenate([blk(pc, j, r * 8, 8) for j in js], axis=1).astype(F32)
                    u = paced(w_ld[pl.ds(r * 16, 16), :] - pb((0, 7, 8)) * d16, t)
                    l = paced(w_ld[pl.ds(HK + r * 16, 16), :] - pb((1, 2, 9)) * d16, t)
                    nb = 8 if h == U - 1 and r * 16 >= (4 - NAT) * 128 else 7
                    dc[pl.ds(r * 8, 8), pl.ds(0, 128 * nb)] = pk(jnp.concatenate(bcomb(u[:, :256], l[:, :256])[:nb], axis=1))
                    dc[pl.ds(r * 8, 8), pl.ds(1024, 256)] = pk(jnp.concatenate([u[:, 256:], l[:, 256:]], axis=1))
            def dQ(h):
                dqt, toks = prob1(k_b[h][...], dc)
                dq = dqt.astype(BF16).T
                dq_b[h][...] = restore(dq)
                st[h]["t"].append(rtok(1, h, 0))
                return toks
            def dK(h):
                q = q_b[h][...]
                nt = 4 - NAT if h == U - 1 else 4
                toks, t = prob2(q.T, dc, dk_b[h], nt)
                st[h]["t"].append(rtok(2, h, 0) if nt == 4 else t)
                for t in range(nt, 4):
                    for base, js in ((0, (0, 7, 8)), (HK, (1, 2, 9))):
                        dk = dg(jnp.concatenate([blk(dc, j, 64 * t, 64) for j in js], axis=1), q, NN)
                        toks += vregs(dk)[::2]
                        if t == 3 and base: dk = jnp.concatenate([dk[:120], dk[120:] + functools.reduce(jnp.add, st[h]["t"])], axis=0)
                        dk_b[h][pl.ds(base + 128 * t, 128), :] = dk.astype(BF16)
                return toks
            return S, X1, X2, O, dV, dP, dQ, dK, Y

        def block(i, ibuf, obuf, U, n, sem, old):
            S, X1, X2, O, dV, dP, dQ, dK, Y = phases(i, ibuf, obuf, U, old)
            for h in range(U):
                dP(h); ts = S(h + 1)
                tv = dV(h); to = O(h)
                Y(h, ts[18:] + tv[:12]); X1(h + 1, tv[27:])
                tq = dQ(h); tk = dK(h)
                X2(h + 1, to[40:] + tq + tk[:72:2])
                for a in range(4): pltpu.make_async_copy(oview(obuf, U, a, h), hsl(hout[a], n + h, 1, ol[a]), sem).start()

        i0 = pl.program_id(0)
        first = [icp(ib0, U0, a, 0, 0, 1, isem.at[2]) for a in range(2)]
        rest = [icp(ib0, U0, a, int(a < 2), int(a < 2), U0, isem.at[3]) for a in range(4)] if U0 else []
        for c in first + rest: c.start()
        fetch(0, 0)
        for c in first: c.wait()
        S, X1, X2 = phases(i0, ib0, ob0.at[0], U0)[:3]
        S(0); X1(0, None); X2(0, None)
        if U0:
            for c in rest: c.wait()
            block(i0, ib0, ob0.at[i0], U0, 0, osem.at[2], ob0.at[lax.shift_right_logical(i0, 20)])

        def body(i, carry):
            p = lax.rem(i, 2)
            wait_all(ib.at[p], isem.at[p])
            @pl.when(i > 1)
            def _():
                wait_all(ob.at[p], osem.at[p])
            @pl.when(i + 1 < NG)
            def _():
                fetch(i + 1, 1 - p)
            block(i, ib.at[p], ob.at[p], U, U0 + i * U, osem.at[p], ob.at[(i + lax.shift_right_logical(i, 20)) & 1])
            return carry
        lax.fori_loop(0, NG, body, 0)
        if U0: wait_all(ob0, osem.at[2])
        for p in range(2): wait_all(ob.at[p], osem.at[p])

    def f(q, k, v, g):
        B, H, Sq, D = q.shape; Sk = k.shape[2]; BH = B * H
        q, k, v, g = [x.reshape(BH * x.shape[2], D) for x in (q, k, v, g)]
        sq = jax.ShapeDtypeStruct((BH * Sq, D), BF16); sk = jax.ShapeDtypeStruct((BH * Sk, D), BF16)
        R = Sq + Sk
        io = [pltpu.VMEM((2, (2 * U + 1) * R, D), BF16), pltpu.VMEM((2, 2 * U * R, D), BF16),
              pltpu.VMEM(((2 * U0 + 1) * R, D), BF16), pltpu.VMEM((1, max(2 * U0 * R, 16), D), BF16)]
        cb = pltpu.VMEM((1, Sk // 4, 1280), U32)
        anyspec = pl.BlockSpec(memory_space=pl.ANY)
        o, dq, dk, dv = pl.pallas_call(kernel, grid=(1,), in_specs=[anyspec] * 4, out_specs=[anyspec] * 4,
            out_shape=[sq, sq, sk, sk], name="mha",
            scratch_shapes=io + [pltpu.VMEM((1, Sk, Sq), F32), pltpu.VMEM((1, Sk, Sq), F32), cb, cb, cb,
                pltpu.SemaphoreType.DMA((4,)), pltpu.SemaphoreType.DMA((3,))],
            compiler_params=pltpu.CompilerParams(dimension_semantics=("arbitrary",), vmem_limit_bytes=100 << 20, disable_bounds_checks=True))(q, k, v, g)
        return o.reshape(B, H, Sq, D), dq.reshape(B, H, Sq, D), dk.reshape(B, H, Sk, D), dv.reshape(B, H, Sk, D)
    return f

_impl = make()

@jax.jit
def pallas_standalone__mha_softmax__near_ridge_kernel(q, k, v, grad_out):
    return _impl(q, k, v, grad_out)
```
